```python
import os as _os
_os.environ.setdefault("JAX_PLATFORMS", "cpu")
import jax
import jax.numpy as jnp

def _softmax(x, axis=-1):
    return jax.nn.softmax(x, axis=axis)
def _gelu(x):
    return jax.nn.gelu(x, approximate=True)
def _silu(x):
    return jax.nn.silu(x)
def _sigmoid(x):
    return jax.nn.sigmoid(x)
def _layernorm(x, axis=-1, eps=1e-5):
    m = jnp.mean(x, axis=axis, keepdims=True)
    v = jnp.var(x, axis=axis, keepdims=True)
    return (x - m) / jnp.sqrt(v + eps)
def _scatter_add(tgt, idx, src, axis=0):
    return tgt.at[idx].add(src)
def _segment_sum(src, seg, n):
    return jax.ops.segment_sum(src, seg, n)
class _Rng:
    def __init__(self, key):
        self._k = key
    def _next(self):
        self._k, sub = jax.random.split(self._k)
        return sub
    def normal(self, shape):
        return jax.random.normal(self._next(), shape, dtype=jnp.bfloat16)
    def randint(self, lo, hi, shape):
        return jax.random.randint(self._next(), shape, lo, hi, dtype=jnp.int32)
    def uniform(self, shape, lo=0.0, hi=1.0):
        return jax.random.uniform(self._next(), shape, jnp.bfloat16, lo, hi)
    def permutation(self, n):
        return jax.random.permutation(self._next(), n)


kernel_name = 'gated_mix__grouped_kv_mqa__ssm_conv_s5__prompt'

def setup_inputs():
    _rng = _Rng(jax.random.key(int.from_bytes(__import__("os").urandom(4), "little")))
    _w = (lambda a: (lambda t: t.astype(jnp.bfloat16) if jnp.issubdtype(t.dtype, jnp.floating) else t)(jnp.asarray(a)))
    def _A_setup():
        B, S, D, H = 1, 2048, 512, 32
        Dh = D // H
        return {
            "x": _w((lambda *s: _rng.normal(s) * 0.05)(B, S, D)),
            "wq": _w((lambda *s: _rng.normal(s) * 1.6)(D, H * Dh)),
            "wk": _w((lambda *s: _rng.normal(s) * 1.6)(D, Dh)),
            "wv": _w((lambda *s: _rng.normal(s) * 0.05)(D, Dh)),
            "wo": _w((lambda *s: _rng.normal(s) * 0.05)(H * Dh, D)),
        }
    _A_in = _A_setup()

    def _B_setup():
        B, S, D = 1, 2048, 512
        P = D
        Lambda_re = -0.5 * jnp.exp((lambda *s: _rng.normal(s) * 0.4)(P))
        Lambda_im = (lambda *s: _rng.normal(s) * 0.4)(P) * 1.0
        B_re = (lambda *s: _rng.normal(s) * 0.4)(P, D) * (D ** -0.5)
        B_im = (lambda *s: _rng.normal(s) * 0.4)(P, D) * (D ** -0.5)
        C_re = (lambda *s: _rng.normal(s) * 0.4)(D, P) * (P ** -0.5)
        C_im = (lambda *s: _rng.normal(s) * 0.4)(D, P) * (P ** -0.5)
        log_dt = (lambda *s: _rng.normal(s) * 0.4)(P) * 0.3 - 2.0
        Dskip = (lambda *s: _rng.normal(s) * 0.4)(D)
        return {
            "x": _w((lambda *s: _rng.normal(s) * 0.05)(B, S, D)),
            "Lambda_re": _w(Lambda_re),
            "Lambda_im": _w(Lambda_im),
            "B_re": _w(B_re),
            "B_im": _w(B_im),
            "C_re": _w(C_re),
            "C_im": _w(C_im),
            "log_dt": _w(log_dt),
            "Dskip": _w(Dskip),
        }
    _B_in = _B_setup()

    return {
        "A_x": _A_in["x"],
        "A_wq": _A_in["wq"],
        "A_wk": _A_in["wk"],
        "A_wv": _A_in["wv"],
        "A_wo": _A_in["wo"],
        "B_x": _B_in["x"],
        "B_Lambda_re": _B_in["Lambda_re"],
        "B_Lambda_im": _B_in["Lambda_im"],
        "B_B_re": _B_in["B_re"],
        "B_B_im": _B_in["B_im"],
        "B_C_re": _B_in["C_re"],
        "B_C_im": _B_in["C_im"],
        "B_log_dt": _B_in["log_dt"],
        "B_Dskip": _B_in["Dskip"],
        "gate_w": _w((lambda *s: _rng.normal(s) * 0.05)(512) * 16.0),
    }

def reference(A_x, A_wq, A_wk, A_wv, A_wo, B_x, B_Lambda_re, B_Lambda_im, B_B_re, B_B_im, B_C_re, B_C_im, B_log_dt, B_Dskip, gate_w):
    def _A_ref(x, wq, wk, wv, wo):
        B, S, D = x.shape
        H = 32
        Dh = D // H
        q = (lambda x, *d: x.transpose(*d))((x @ wq).reshape(B, S, H, Dh), 0, 2, 1, 3)
        k = x @ wk
        v = x @ wv
        scores = jnp.einsum("bhqd,bkd->bhqk", q, k) * (Dh ** -0.5)
        p = _softmax(scores, axis=-1)
        o = jnp.einsum("bhqk,bkd->bhqd", p, v)
        return (lambda x, *d: x.transpose(*d))(o, 0, 2, 1, 3).reshape(B, S, H * Dh) @ wo

    def _B_ref(x, Lambda_re, Lambda_im, B_re, B_im, C_re, C_im, log_dt, Dskip):
        Bsz, L, H = x.shape
        Lam = Lambda_re + 1j * Lambda_im
        Bmat = B_re + 1j * B_im
        Cmat = C_re + 1j * C_im
        dt = jnp.exp(log_dt)
        Lam_bar = jnp.exp(dt * Lam)
        B_bar = ((Lam_bar - 1.0) / Lam)[:, None] * Bmat
        Bu = jnp.einsum("bld,pd->blp", x + 0j, B_bar)
        h = jnp.zeros_like(Bu[:, 0, :])
        hs = []
        for t in range(L):
            h = Lam_bar[None, :] * h + Bu[:, t, :]
            hs.append(h)
        hseq = jnp.stack(hs, 1)
        y = 2.0 * jnp.einsum("blp,dp->bld", hseq, Cmat).real + x * Dskip[None, None, :]
        return y

    x = A_x
    g = _sigmoid((x * gate_w).sum(-1, keepdims=True))
    a = _A_ref(x, A_wq, A_wk, A_wv, A_wo)
    b = _B_ref(x, B_Lambda_re, B_Lambda_im, B_B_re, B_B_im, B_C_re, B_C_im, B_log_dt, B_Dskip)
    return g * a + (1 - g) * b
```

```python
import jax
import jax.numpy as jnp
import jax.experimental.pallas as pl
import jax.experimental.pallas.tpu as pltpu

S, D, H, DH, P = 2048, 512, 32, 16, 512
TQ = 512
NT = S // TQ
RSEG = 16
NSEG = TQ // RSEG
SCH = 64
NSCH = S // SCH
VX_ROWS = DH + 8
_F32 = jnp.float32
_BF16 = jnp.bfloat16


def _dot(a, b, ca, cb):
    return jax.lax.dot_general(a, b, (((ca,), (cb,)), ((), ())),
                               preferred_element_type=_F32)


def _kernel(x_ref, wq_ref, wk_ref, wv_ref, wo_ref,
            lre_ref, lim_ref, bre_ref, bim_ref, cre_ref, cim_ref,
            ldt_ref, dsk_ref, gw_ref,
            out_ref,
            k_s, vx_s, bb_s, pw_s, carry_s,
            s0_s, s1_s, p0_s, p1_s, m0_s, m1_s,
            qT_s, oT_s, scan_s):
    s_s = (s0_s, s1_s)
    p_s = (p0_s, p1_s)
    m_s = (m0_s, m1_s)
    i = pl.program_id(0)

    @pl.when(i == 0)
    def _prologue():
        xf = x_ref[...]
        k_s[...] = _dot(xf, wk_ref[...], 1, 0).astype(_BF16)
        vx_s[0:DH, :] = _dot(wv_ref[...], xf, 0, 1).astype(_BF16)
        row = jax.lax.broadcasted_iota(jnp.int32, (VX_ROWS - DH, S), 0)
        vx_s[DH:VX_ROWS, :] = jnp.where(row == 0, 1.0, 0.0).astype(_BF16)
        lre = lre_ref[...].reshape(1, P).astype(_F32)
        lim = lim_ref[...].reshape(1, P).astype(_F32)
        dt = jnp.exp(ldt_ref[...].reshape(1, P).astype(_F32))
        are = dt * lre
        aim = dt * lim
        e = jnp.exp(are)
        lb_re = e * jnp.cos(aim)
        lb_im = e * jnp.sin(aim)
        nre = lb_re - 1.0
        nim = lb_im
        den = lre * lre + lim * lim
        c_re = (nre * lre + nim * lim) / den
        c_im = (nim * lre - nre * lim) / den
        c_re_col = c_re.reshape(P, 1)
        c_im_col = c_im.reshape(P, 1)
        b_re = bre_ref[...].astype(_F32)
        b_im = bim_ref[...].astype(_F32)
        bb_s[0] = (c_re_col * b_re - c_im_col * b_im).astype(_BF16)
        bb_s[1] = (c_re_col * b_im + c_im_col * b_re).astype(_BF16)
        jj = jax.lax.broadcasted_iota(jnp.int32, (RSEG, P), 0).astype(_F32) + 1.0
        ej = jnp.exp(jj * are)
        angle = jj * aim
        pw_s[0] = ej * jnp.cos(angle)
        pw_s[1] = ej * jnp.sin(angle)
        carry_s[...] = jnp.zeros(carry_s.shape, _F32)

    x_t = x_ref[pl.ds(i * TQ, TQ), :]

    qT_s[...] = (_dot(wq_ref[...], x_t, 0, 1) * 0.25).astype(_BF16)

    def scores_max(h, buf):
        qh = qT_s[pl.ds(h * DH, DH), :]
        acc = None
        for c in range(NSCH):
            r = _dot(k_s[pl.ds(c * SCH, SCH), :], qh, 1, 0)
            s_s[buf][pl.ds(c * SCH, SCH), :] = r
            acc = r if acc is None else jnp.maximum(acc, r)
        m_s[buf][...] = jnp.max(acc, axis=0, keepdims=True)

    def softmax_exp(buf):
        m = m_s[buf][...]
        for j in range(NSCH):
            p_s[buf][pl.ds(j * SCH, SCH), :] = jnp.exp(
                s_s[buf][pl.ds(j * SCH, SCH), :] - m).astype(_BF16)

    def pv(h, buf):
        oh = _dot(vx_s[...], p_s[buf][...], 1, 0)
        oT_s[pl.ds(h * DH, DH), :] = (
            oh[0:DH, :] * (1.0 / oh[DH:DH + 1, :])).astype(_BF16)

    scores_max(0, 0)
    scores_max(1, 1)
    softmax_exp(0)

    def pair(j, c):
        t = 2 * j + 1
        scores_max(t + 1, 0)
        pv(t - 1, 0)
        softmax_exp(1)
        scores_max(t + 2, 1)
        pv(t, 1)
        softmax_exp(0)
        return c

    jax.lax.fori_loop(0, H // 2 - 1, pair, 0)
    pv(H - 2, 0)
    softmax_exp(1)
    pv(H - 1, 1)
    a_att = _dot(oT_s[...], wo_ref[...], 0, 0)

    scan_s[0, 0] = _dot(x_t, bb_s[0], 1, 1)
    scan_s[0, 1] = _dot(x_t, bb_s[1], 1, 1)
    loc = jax.lax.broadcasted_iota(jnp.int32, (TQ, P), 0) % RSEG
    d = 1
    src = 0
    while d < RSEG:
        dst = 1 - src
        are_d = pw_s[0, pl.ds(d - 1, 1), :]
        aim_d = pw_s[1, pl.ds(d - 1, 1), :]
        re = scan_s[src, 0]
        im = scan_s[src, 1]
        valid = loc >= d
        sre = jnp.where(valid, pltpu.roll(re, d, 0), 0.0)
        sim = jnp.where(valid, pltpu.roll(im, d, 0), 0.0)
        scan_s[dst, 0] = re + are_d * sre - aim_d * sim
        scan_s[dst, 1] = im + are_d * sim + aim_d * sre
        src = dst
        d *= 2
    c_re = carry_s[0]
    c_im = carry_s[1]
    pre = pw_s[0]
    pim = pw_s[1]
    for g in range(NSEG):
        rows = pl.ds(g * RSEG, RSEG)
        h_re = scan_s[src, 0, rows, :] + pre * c_re - pim * c_im
        h_im = scan_s[src, 1, rows, :] + pre * c_im + pim * c_re
        scan_s[src, 0, rows, :] = h_re
        scan_s[src, 1, rows, :] = h_im
        c_re = h_re[RSEG - 1:RSEG, :]
        c_im = h_im[RSEG - 1:RSEG, :]
    carry_s[0] = c_re
    carry_s[1] = c_im
    h_re = scan_s[src, 0]
    h_im = scan_s[src, 1]
    xtf = x_t.astype(_F32)
    y = 2.0 * (_dot(h_re.astype(_BF16), cre_ref[...], 1, 1)
               - _dot(h_im.astype(_BF16), cim_ref[...], 1, 1))
    y = y + xtf * dsk_ref[...].reshape(1, D).astype(_F32)

    g = jax.nn.sigmoid(jnp.sum(xtf * gw_ref[...].reshape(1, D).astype(_F32),
                               axis=1, keepdims=True))
    out_ref[...] = g * a_att + (1.0 - g) * y


@jax.jit
def pallas_gated_mix__grouped_kv_mqa__ssm_conv_s5__prompt_kernel(
    A_x: jax.Array,
    A_wq: jax.Array,
    A_wk: jax.Array,
    A_wv: jax.Array,
    A_wo: jax.Array,
    B_x: jax.Array,
    B_Lambda_re: jax.Array,
    B_Lambda_im: jax.Array,
    B_B_re: jax.Array,
    B_B_im: jax.Array,
    B_C_re: jax.Array,
    B_C_im: jax.Array,
    B_log_dt: jax.Array,
    B_Dskip: jax.Array,
    gate_w: jax.Array,
):
    B, S_, D_ = A_x.shape
    assert (B, S_, D_) == (1, S, D)
    x2 = A_x.reshape(S, D)

    def full(shape):
        return pl.BlockSpec(shape, lambda i: tuple(0 for _ in shape))

    in_specs = [
        full((S, D)),
        full((D, H * DH)),
        full((D, DH)),
        full((D, DH)),
        full((H * DH, D)),
        full((P,)), full((P,)),
        full((P, D)), full((P, D)),
        full((D, P)), full((D, P)),
        full((P,)),
        full((D,)),
        full((D,)),
    ]
    out = pl.pallas_call(
        _kernel,
        grid=(NT,),
        in_specs=in_specs,
        out_specs=pl.BlockSpec((TQ, D), lambda i: (i, 0)),
        out_shape=jax.ShapeDtypeStruct((S, D), _F32),
        scratch_shapes=[
            pltpu.VMEM((S, DH), _BF16),
            pltpu.VMEM((VX_ROWS, S), _BF16),
            pltpu.VMEM((2, P, D), _BF16),
            pltpu.VMEM((2, RSEG, P), _F32),
            pltpu.VMEM((2, 1, P), _F32),
            pltpu.VMEM((S, TQ), _F32),
            pltpu.VMEM((S, TQ), _F32),
            pltpu.VMEM((S, TQ), _BF16),
            pltpu.VMEM((S, TQ), _BF16),
            pltpu.VMEM((1, TQ), _F32),
            pltpu.VMEM((1, TQ), _F32),
            pltpu.VMEM((D, TQ), _BF16),
            pltpu.VMEM((D, TQ), _BF16),
            pltpu.VMEM((2, 2, TQ, P), _F32),
        ],
        compiler_params=pltpu.CompilerParams(
            vmem_limit_bytes=100 * 1024 * 1024,
        ),
    )(x2, A_wq, A_wk, A_wv, A_wo,
      B_Lambda_re, B_Lambda_im, B_B_re, B_B_im, B_C_re, B_C_im,
      B_log_dt, B_Dskip, gate_w)
    return out.reshape(B, S, D)
```
